```python
import os as _os
_os.environ.setdefault("JAX_PLATFORMS", "cpu")
import jax
import jax.numpy as jnp

def _softmax(x, axis=-1):
    return jax.nn.softmax(x, axis=axis)
def _gelu(x):
    return jax.nn.gelu(x, approximate=True)
def _silu(x):
    return jax.nn.silu(x)
def _sigmoid(x):
    return jax.nn.sigmoid(x)
def _layernorm(x, axis=-1, eps=1e-5):
    m = jnp.mean(x, axis=axis, keepdims=True)
    v = jnp.var(x, axis=axis, keepdims=True)
    return (x - m) / jnp.sqrt(v + eps)
def _scatter_add(tgt, idx, src, axis=0):
    return tgt.at[idx].add(src)
def _segment_sum(src, seg, n):
    return jax.ops.segment_sum(src, seg, n)
class _Rng:
    def __init__(self, key):
        self._k = key
    def _next(self):
        self._k, sub = jax.random.split(self._k)
        return sub
    def normal(self, shape):
        return jax.random.normal(self._next(), shape, dtype=jnp.bfloat16)
    def randint(self, lo, hi, shape):
        return jax.random.randint(self._next(), shape, lo, hi, dtype=jnp.int32)
    def uniform(self, shape, lo=0.0, hi=1.0):
        return jax.random.uniform(self._next(), shape, jnp.bfloat16, lo, hi)
    def permutation(self, n):
        return jax.random.permutation(self._next(), n)


kernel_name = 'sequential_preLN__softmax_full_mha__glu_gated_swiglu__prompt'

def setup_inputs():
    _rng = _Rng(jax.random.key(int.from_bytes(__import__("os").urandom(4), "little")))
    _w = (lambda a: (lambda t: t.astype(jnp.bfloat16) if jnp.issubdtype(t.dtype, jnp.floating) else t)(jnp.asarray(a)))
    def _A_setup():
        B, S, D = 1, 2048, 640
        return {
            "x": _w((lambda *s: _rng.normal(s) * 0.05)(B, S, D)),
            "wqkv": _w((lambda *s: _rng.normal(s) * 0.05)(D, 3 * D)),
            "wo": _w((lambda *s: _rng.normal(s) * 0.05)(D, D)),
        }
    _A_in = _A_setup()

    def _B_setup():
        B, S, D, F = 1, 2048, 640, 1728
        return {
            "x": _w((lambda *s: _rng.normal(s) * 0.05)(B, S, D)),
            "w1": _w((lambda *s: _rng.normal(s) * 0.05)(D, F) * (2.0 / D) ** 0.5),
            "w3": _w((lambda *s: _rng.normal(s) * 0.05)(D, F) * (2.0 / D) ** 0.5),
            "w2": _w((lambda *s: _rng.normal(s) * 0.05)(F, D) * (2.0 / F) ** 0.5),
        }
    _B_in = _B_setup()

    return {
        "A_x": _A_in["x"],
        "A_wqkv": _A_in["wqkv"],
        "A_wo": _A_in["wo"],
        "B_x": _B_in["x"],
        "B_w1": _B_in["w1"],
        "B_w3": _B_in["w3"],
        "B_w2": _B_in["w2"],
    }

def reference(A_x, A_wqkv, A_wo, B_x, B_w1, B_w3, B_w2):
    def _A_ref(x, wqkv, wo):
        B, S, D = x.shape
        H = 32; Dh = D // H
        qkv = (lambda x, *d: x.transpose(*d))((x @ wqkv).reshape(B, S, 3, H, Dh), 2, 0, 3, 1, 4)
        q, k, v = qkv[0], qkv[1], qkv[2]
        scale = Dh ** -0.5
        scores = jnp.einsum("bhqd,bhkd->bhqk", q, k) * scale
        p = _softmax(scores, axis=-1)
        o = jnp.einsum("bhqk,bhkd->bhqd", p, v)
        return (lambda x, *d: x.transpose(*d))(o, 0, 2, 1, 3).reshape(B, S, D) @ wo

    def _B_ref(x, w1, w3, w2):
        gate = jnp.einsum("bsd,df->bsf", x, w1)
        up = jnp.einsum("bsd,df->bsf", x, w3)
        h = _silu(gate) * up
        out = jnp.einsum("bsf,fd->bsd", h, w2)
        return out

    x = A_x
    h = x + _A_ref(_layernorm(x, axis=-1), A_wqkv, A_wo)
    h2 = h + _B_ref(_layernorm(h, axis=-1), B_w1, B_w3, B_w2)
    return h2
```

```python
import jax
import jax.numpy as jnp
from jax.experimental import pallas as pl
from jax.experimental.pallas import tpu as pltpu

BF16 = jnp.bfloat16
F32 = jnp.float32

S = 2048
D = 640
H = 32
DH = D // H
F = 1728
NG = 6
HG = 6
VR = 24
EPS = 1e-5
NT = (((1,), (1,)), ((), ()))
QSCALE = (DH ** -0.5) * 1.4426950408889634

RC = 512
KC = 128
QS = 512
FC = 256


def _layernorm(x):
    mu = jnp.mean(x, axis=-1, keepdims=True)
    xc = x - mu
    var = jnp.mean(xc * xc, axis=-1, keepdims=True)
    return xc * jax.lax.rsqrt(var + EPS)


def _kernel(x_hbm, wqkv_hbm, wo_hbm, w1_hbm, w3_hbm, w2_hbm, out_hbm,
            x_v, wqkv_v, wo_v, w1_v, w3_v, w2_v, wqvT, kg, qgT, vpad, opad, sb0, sb1, ostage,
            in_sem, x_sem, out_sem):
    nrc = S // RC

    x_cp = [pltpu.make_async_copy(x_hbm.at[pl.ds(r * RC, RC)], x_v.at[pl.ds(r * RC, RC)], x_sem.at[r])
            for r in range(nrc)]
    w_cp = [pltpu.make_async_copy(src, dst, in_sem.at[i]) for i, (src, dst) in enumerate(
        ((wqkv_hbm, wqkv_v), (wo_hbm, wo_v), (w1_hbm, w1_v), (w3_hbm, w3_v), (w2_hbm, w2_v)))]
    x_cp[0].start()
    w_cp[0].start()
    for c in x_cp[1:]:
        c.start()
    for c in w_cp[1:]:
        c.start()

    w_cp[0].wait()
    for i, c0 in enumerate((0, 2 * D)):
        wqvT[i * D:(i + 1) * D, :] = wqkv_v[:, c0:c0 + D].astype(F32).T.astype(BF16)

    def qkv_chunk(r, carry):
        r0 = pl.multiple_of(r * RC, RC)
        pltpu.make_async_copy(x_hbm.at[pl.ds(r0, RC)], x_v.at[pl.ds(r0, RC)], x_sem.at[r]).wait()
        xb = _layernorm(x_v[pl.ds(r0, RC), :].astype(F32)).astype(BF16)
        k = jnp.dot(xb, wqkv_v[:, D:2 * D], preferred_element_type=F32).astype(BF16)
        for g in range(NG):
            lo = HG * DH * g
            if lo + 128 <= D:
                kg[g, pl.ds(r0, RC), :] = k[:, lo:lo + 128]
            else:
                kg[g, pl.ds(r0, RC), :] = jnp.concatenate(
                    [k[:, lo:D], jnp.zeros((RC, lo + 128 - D), BF16)], axis=1)
        qv = jax.lax.dot_general(wqvT[...], xb, (((1,), (1,)), ((), ())), preferred_element_type=F32)
        qT = qv[0:D] * QSCALE
        for g in range(NG):
            lo = HG * DH * g
            if lo + 128 <= D:
                qgT[g, :, pl.ds(r0, RC)] = qT[lo:lo + 128].astype(BF16)
            else:
                qgT[g, :, pl.ds(r0, RC)] = jnp.concatenate(
                    [qT[lo:D], jnp.zeros((lo + 128 - D, RC), F32)], axis=0).astype(BF16)
        vT = qv[D:2 * D].astype(BF16).astype(F32)
        vT = jnp.concatenate([vT, jnp.zeros((8, RC), F32)], axis=0)
        row = jax.lax.broadcasted_iota(jnp.int32, (VR, RC), 0)
        fill = jnp.where(row == DH, 1.0, 0.0).astype(F32)
        for h in range(H):
            vpad[h, :, pl.ds(r0, RC)] = jnp.where(row < DH, vT[DH * h:DH * h + VR], fill)
        return carry

    jax.lax.fori_loop(0, nrc, qkv_chunk, 0)

    nqs = S // QS
    nkc = S // KC

    def masked_q(h, j):
        g = h // HG
        lo = (h - g * HG) * DH
        row = jax.lax.broadcasted_iota(jnp.int32, (128, QS), 0)
        q = qgT[g, :, j * QS:(j + 1) * QS]
        return jnp.where((row >= lo) & (row < lo + DH), q, jnp.zeros_like(q))

    def score_chunk(h, qm, c, j, sb, mx):
        s = jnp.dot(kg[h // HG, c * KC:(c + 1) * KC, :], qm, preferred_element_type=F32)
        sb[c * KC:(c + 1) * KC, j * QS:(j + 1) * QS] = s
        bm = jnp.max(s.reshape(KC // 8, 8, QS), axis=0)
        return bm if mx is None else jnp.maximum(mx, bm)

    def pv_chunk(h, c, j, sb, m8, o):
        s = sb[c * KC:(c + 1) * KC, j * QS:(j + 1) * QS]
        p = jnp.exp2(s.reshape(KC // 8, 8, QS) - m8[None]).reshape(KC, QS).astype(BF16)
        d = jnp.dot(vpad[h, :, c * KC:(c + 1) * KC], p, preferred_element_type=F32)
        return d if o is None else o + d

    def fin_max(mx):
        return jnp.broadcast_to(jnp.max(mx, axis=0, keepdims=True), (8, QS))

    def fin_out(h, j, o):
        opad[h, :, j * QS:(j + 1) * QS] = o * (1.0 / o[DH:DH + 1, :])

    def step(h, m_cur, sb_cur, sb_nxt):
        m_nxt = []
        for j in range(nqs):
            qm = masked_q(h + 1, j)
            mx, o = None, None
            for c in range(nkc):
                mx = score_chunk(h + 1, qm, c, j, sb_nxt, mx)
                o = pv_chunk(h, c, j, sb_cur, m_cur[j], o)
            fin_out(h, j, o)
            m_nxt.append(fin_max(mx))
        return tuple(m_nxt)

    m0 = []
    for j in range(nqs):
        qm = masked_q(0, j)
        mx = None
        for c in range(nkc):
            mx = score_chunk(0, qm, c, j, sb0, mx)
        m0.append(fin_max(mx))

    def head_body(h, m_cur):
        return jax.lax.cond(h % 2 == 0,
                            lambda: step(h, m_cur, sb0, sb1),
                            lambda: step(h, m_cur, sb1, sb0))

    m_last = jax.lax.fori_loop(0, H - 1, head_body, tuple(m0))
    for j in range(nqs):
        o = None
        for c in range(nkc):
            o = pv_chunk(H - 1, c, j, sb1, m_last[j], o)
        fin_out(H - 1, j, o)

    for c in w_cp[1:]:
        c.wait()

    fchunks = [(f0, min(FC, F - f0)) for f0 in range(0, F, FC)]

    def mlp_chunk(r, carry):
        r0 = pl.multiple_of(r * RC, RC)
        slot = r % 2
        oT = jnp.concatenate([opad[h, 0:DH, pl.ds(r0, RC)] for h in range(H)], axis=0)
        o = oT.T.astype(BF16)
        hres = x_v[pl.ds(r0, RC), :].astype(F32) + jnp.dot(o, wo_v[...], preferred_element_type=F32)
        hn = _layernorm(hres).astype(BF16)
        acc = hres
        for f0, fw in fchunks:
            gate = jax.lax.dot_general(hn, w1_v[f0:f0 + fw, :], NT, preferred_element_type=F32)
            up = jax.lax.dot_general(hn, w3_v[f0:f0 + fw, :], NT, preferred_element_type=F32)
            act = (gate * jax.nn.sigmoid(gate) * up).astype(BF16)
            acc = acc + jnp.dot(act, w2_v[f0:f0 + fw, :], preferred_element_type=F32)

        @pl.when(r >= 2)
        def _():
            pltpu.make_async_copy(ostage.at[slot], out_hbm.at[pl.ds(r0, RC)], out_sem.at[slot]).wait()

        ostage[slot] = acc.astype(BF16)
        pltpu.make_async_copy(ostage.at[slot], out_hbm.at[pl.ds(r0, RC)], out_sem.at[slot]).start()
        return carry

    jax.lax.fori_loop(0, nrc, mlp_chunk, 0)
    for slot in range(2):
        pltpu.make_async_copy(ostage.at[slot], out_hbm.at[pl.ds(0, RC)], out_sem.at[slot]).wait()


@jax.jit
def pallas_sequential_preLN__softmax_full_mha__glu_gated_swiglu__prompt_kernel(
    A_x: jax.Array,
    A_wqkv: jax.Array,
    A_wo: jax.Array,
    B_x: jax.Array,
    B_w1: jax.Array,
    B_w3: jax.Array,
    B_w2: jax.Array,
):
    del B_x
    b, s, d = A_x.shape
    assert (b, s, d) == (1, S, D)
    any_spec = pl.BlockSpec(memory_space=pltpu.MemorySpace.HBM)
    out = pl.pallas_call(
        _kernel,
        out_shape=jax.ShapeDtypeStruct((S, D), A_x.dtype),
        in_specs=[any_spec] * 6,
        out_specs=any_spec,
        scratch_shapes=[
            pltpu.VMEM((S, D), BF16),
            pltpu.VMEM((D, 3 * D), BF16),
            pltpu.VMEM((D, D), BF16),
            pltpu.VMEM((F, D), BF16),
            pltpu.VMEM((F, D), BF16),
            pltpu.VMEM((F, D), BF16),
            pltpu.VMEM((2 * D, D), BF16),
            pltpu.VMEM((NG, S, 128), BF16),
            pltpu.VMEM((NG, 128, S), BF16),
            pltpu.VMEM((H, VR, S), F32),
            pltpu.VMEM((H, VR, S), F32),
            pltpu.VMEM((S, S), F32),
            pltpu.VMEM((S, S), F32),
            pltpu.VMEM((2, RC, D), BF16),
            pltpu.SemaphoreType.DMA((5,)),
            pltpu.SemaphoreType.DMA((S // RC,)),
            pltpu.SemaphoreType.DMA((2,)),
        ],
        compiler_params=pltpu.CompilerParams(vmem_limit_bytes=110 * 2 ** 20),
    )(A_x.reshape(S, D), A_wqkv, A_wo, B_w1.T, B_w3.T, B_w2)
    return out.reshape(b, s, d)
```

```python
import jax
import jax.numpy as jnp
from jax.experimental import pallas as pl
from jax.experimental.pallas import tpu as pltpu

BF16 = jnp.bfloat16
F32 = jnp.float32

S = 2048
D = 640
H = 32
DH = D // H
F = 1728
LANES = 128
HG = 6
NG = -(-H // HG)
VR = 24
EPS = 1e-5
QSCALE = (DH ** -0.5) * 1.4426950408889634
NT = (((1,), (1,)), ((), ()))

RC = 512
NRC = S // RC
KC = 256
QS = 256
FC = 512
LNR = 32


def _window_rows(t, g, axis):
    lo = HG * DH * g
    hi = min(lo + LANES, D)
    w = jax.lax.slice_in_dim(t, lo, hi, axis=axis)
    if hi - lo < LANES:
        pad = list(t.shape)
        pad[axis] = lo + LANES - hi
        w = jnp.concatenate([w, jnp.zeros(pad, t.dtype)], axis=axis)
    return w


def _kernel(x_hbm, wqkv_hbm, wo_hbm, w1T_hbm, w3T_hbm, w2_hbm, out_hbm,
            x_v, xn, kraw, wqv_v, wk_v, wo_v, w1T, w3T, w2_v, wqvT, woT, w2T,
            kg, qgT, vpad, opad, sb, msc, qm0, ostage,
            w_sem, x_sem, out_sem):

    def x_cp(r):
        return pltpu.make_async_copy(x_hbm.at[pl.ds(r * RC, RC)], x_v.at[pl.ds(r * RC, RC)], x_sem.at[r])

    def out_cp(r0, i):
        return pltpu.make_async_copy(
            ostage.at[pl.ds(r0, LANES)], out_hbm.at[pl.ds(r0, LANES)], out_sem.at[i])

    wk_cp = pltpu.make_async_copy(wqkv_hbm.at[:, D:2 * D], wk_v, w_sem.at[0])
    wq_cp = pltpu.make_async_copy(wqkv_hbm.at[:, 0:D], wqv_v.at[0:D], w_sem.at[1])
    wv_cp = pltpu.make_async_copy(wqkv_hbm.at[:, 2 * D:3 * D], wqv_v.at[D:2 * D], w_sem.at[2])
    late_cp = [pltpu.make_async_copy(src, dst, w_sem.at[3 + i]) for i, (src, dst) in enumerate(
        ((wo_hbm, wo_v), (w2_hbm, w2_v), (w1T_hbm, w1T), (w3T_hbm, w3T)))]

    x_cp(0).start()
    wk_cp.start()
    x_cp(0).wait()
    x_cp(1).start()
    wk_cp.wait()

    def k_chunk(r, carry, transpose_w):
        r0 = pl.multiple_of(r * RC, RC)

        @pl.when(r >= 1)
        def _():
            x_cp(r).wait()

        @pl.when((r >= 1) & (r + 1 < NRC))
        def _():
            x_cp(r + 1).start()

        if not transpose_w:
            @pl.when(r == 0)
            def _():
                wq_cp.start()
                wv_cp.start()

        raw = jnp.dot(x_v[pl.ds(r0, RC), :], wk_v[...], preferred_element_type=F32)
        colsum = jnp.sum(wk_v[...].astype(F32), axis=0, keepdims=True)
        ks = []
        for i in range(RC // LNR):
            rows = pl.ds(r0 + i * LNR, LNR)
            xf = x_v[rows, :].astype(F32)
            mu = jnp.mean(xf, axis=-1, keepdims=True)
            xc = xf - mu
            rstd = jax.lax.rsqrt(jnp.mean(xc * xc, axis=-1, keepdims=True) + EPS)
            xn[rows, :] = (xc * rstd).astype(BF16)
            ks.append(((raw[i * LNR:(i + 1) * LNR] - mu * colsum) * rstd).astype(BF16))
        kraw[pl.ds(r0, RC), :] = jnp.concatenate(ks, axis=0)
        if transpose_w:
            wr = pl.ds(pl.multiple_of((r - NRC // 2) * D, D), D)
            wqvT[wr, :] = wqv_v[wr, :].T
        return carry

    jax.lax.fori_loop(0, NRC // 2, lambda r, c: k_chunk(r, c, False), 0)
    wq_cp.wait()
    wv_cp.wait()
    jax.lax.fori_loop(NRC // 2, NRC, lambda r, c: k_chunk(r, c, True), 0)
    for c in late_cp:
        c.start()

    def qv_chunk(r, carry):
        r0 = pl.multiple_of(r * RC, RC)
        cols = pl.ds(r0, RC)
        qv = jax.lax.dot_general(wqvT[...], xn[cols, :], NT, preferred_element_type=F32)
        for i in range(RC // LNR):
            rows = pl.ds(r0 + i * LNR, LNR)
            k = kraw[rows, :]
            for g in range(NG):
                kg[g, rows, :] = _window_rows(k, g, 1)
        qT = qv[0:D] * QSCALE
        for g in range(NG):
            qgT[g, :, cols] = _window_rows(qT, g, 0).astype(BF16)
        vT = qv[D:2 * D].astype(BF16).astype(F32)
        vT = jnp.concatenate([vT, jnp.zeros((8, RC), F32)], axis=0)
        row = jax.lax.broadcasted_iota(jnp.int32, (VR, RC), 0)
        fill = jnp.where(row == DH, 1.0, 0.0).astype(F32)
        for h in range(H):
            vpad[h, :, cols] = jnp.where(row < DH, vT[DH * h:DH * h + VR], fill)
        return carry

    jax.lax.fori_loop(0, NRC, qv_chunk, 0)

    nqs = S // QS
    nkc = S // KC

    def masked_q(g, lo, j):
        row = jax.lax.broadcasted_iota(jnp.int32, (LANES, QS), 0)
        q = qgT[g, :, j * QS:(j + 1) * QS]
        return jnp.where((row >= lo) & (row < lo + DH), q, jnp.zeros_like(q))

    def score_chunk(g, qm, c, j, mx):
        s = jnp.dot(kg[g, c * KC:(c + 1) * KC, :], qm, preferred_element_type=F32)
        sb[c * KC:(c + 1) * KC, j * QS:(j + 1) * QS] = s
        bm = jnp.max(s.reshape(KC // 8, 8, QS), axis=0)
        return bm if mx is None else jnp.maximum(mx, bm)

    def row_max(j):
        m = jnp.max(msc[:, j * QS:(j + 1) * QS], axis=0, keepdims=True)
        return jnp.broadcast_to(m, (8, QS))

    def probs(c, j, m8):
        s = sb[c * KC:(c + 1) * KC, j * QS:(j + 1) * QS]
        return jnp.exp2(s.reshape(KC // 8, 8, QS) - m8[None]).reshape(KC, QS).astype(BF16)

    def pv_chunk(h, c, p, o):
        d = jnp.dot(vpad[h, :, c * KC:(c + 1) * KC], p, preferred_element_type=F32)
        return d if o is None else o + d

    def step(h, carry):
        g, lo = carry
        m_cur = [row_max(j) for j in range(nqs)]
        m_nxt = []
        for j in range(nqs):
            qm = qm0[...] if j == 0 else masked_q(g, lo, j)
            mx, o = None, None
            for c in range(nkc):
                p = probs(c, j, m_cur[j])
                mx = score_chunk(g, qm, c, j, mx)
                o = pv_chunk(h, c, p, o)
            opad[h, :, j * QS:(j + 1) * QS] = o
            m_nxt.append(mx)
        for j in range(nqs):
            msc[:, j * QS:(j + 1) * QS] = m_nxt[j]
        wrap = lo + DH >= HG * DH
        g2, lo2 = jnp.where(wrap, g + 1, g), jnp.where(wrap, 0, lo + DH)
        qm0[...] = masked_q(jnp.minimum(g2, NG - 1), lo2, 0)
        return g2, lo2

    for j in range(nqs):
        qm = masked_q(0, 0, j)
        mx = None
        for c in range(nkc):
            mx = score_chunk(0, qm, c, j, mx)
        msc[:, j * QS:(j + 1) * QS] = mx
    qm0[...] = masked_q(0, DH, 0)

    jax.lax.fori_loop(0, H - 1, step, (jnp.int32(0), jnp.int32(DH)))

    for c in late_cp:
        c.wait()
    tpieces = [(wo_v, woT, a, LANES) for a in range(0, D, LANES)]
    tpieces += [(w2_v, w2T, a, min(LANES, F - a)) for a in range(0, F, LANES)]
    n = 0
    for j in range(nqs):
        m8 = row_max(j)
        o = None
        for c in range(nkc):
            o = pv_chunk(H - 1, c, probs(c, j, m8), o)
            if n % 3 == 1 and tpieces:
                src, dst, a, w = tpieces.pop(0)
                dst[:, a:a + w] = src[a:a + w, :].T
            n += 1
        opad[H - 1, :, j * QS:(j + 1) * QS] = o
    assert not tpieces

    fchunks = [(f0, min(FC, F - f0)) for f0 in range(0, F, FC)]

    def mlp_chunk(r, carry):
        r0 = pl.multiple_of(r * RC, RC)
        cols = pl.ds(r0, RC)
        pieces = []
        for h in range(H):
            oh = opad[h, :, cols]
            pieces.append(oh[0:DH] * (1.0 / oh[DH:DH + 1]))
        oT = jnp.concatenate(pieces, axis=0).astype(BF16)
        hT = x_v[cols, :].astype(F32).T + jnp.dot(woT[...], oT, preferred_element_type=F32)
        mu = jnp.mean(hT, axis=0, keepdims=True)
        hc = hT - mu
        var = jnp.mean(hc * hc, axis=0, keepdims=True)
        hn = (hc * jax.lax.rsqrt(var + EPS)).astype(BF16)

        def gate_up(i):
            f0, fw = fchunks[i]
            w = jnp.concatenate([w1T[f0:f0 + fw, :], w3T[f0:f0 + fw, :]], axis=0)
            gu = jnp.dot(w, hn, preferred_element_type=F32)
            return gu[0:fw], gu[fw:2 * fw]

        acc = hT
        cur = gate_up(0)
        for i, (f0, fw) in enumerate(fchunks):
            nxt = gate_up(i + 1) if i + 1 < len(fchunks) else None
            g, u = cur
            act = (g * jax.nn.sigmoid(g) * u).astype(BF16)
            acc = acc + jnp.dot(w2T[:, f0:f0 + fw], act, preferred_element_type=F32)
            cur = nxt
        for i in range(RC // LANES):
            rr = pl.multiple_of(r0 + i * LANES, LANES)
            ostage[pl.ds(rr, LANES), :] = acc[:, i * LANES:(i + 1) * LANES].T.astype(BF16)
            out_cp(rr, r * (RC // LANES) + i).start()
        return carry

    jax.lax.fori_loop(0, NRC, mlp_chunk, 0)
    for i in range(S // LANES):
        out_cp(i * LANES, i).wait()


@jax.jit
def pallas_sequential_preLN__softmax_full_mha__glu_gated_swiglu__prompt_kernel(
    A_x: jax.Array,
    A_wqkv: jax.Array,
    A_wo: jax.Array,
    B_x: jax.Array,
    B_w1: jax.Array,
    B_w3: jax.Array,
    B_w2: jax.Array,
):
    del B_x
    b, s, d = A_x.shape
    assert (b, s, d) == (1, S, D) and B_w1.shape == (D, F)
    hbm = pl.BlockSpec(memory_space=pltpu.MemorySpace.HBM)
    out = pl.pallas_call(
        _kernel,
        out_shape=jax.ShapeDtypeStruct((S, D), A_x.dtype),
        in_specs=[hbm] * 6,
        out_specs=hbm,
        scratch_shapes=[
            pltpu.VMEM((S, D), BF16),
            pltpu.VMEM((S, D), BF16),
            pltpu.VMEM((S, D), BF16),
            pltpu.VMEM((2 * D, D), BF16),
            pltpu.VMEM((D, D), BF16),
            pltpu.VMEM((D, D), BF16),
            pltpu.VMEM((F, D), BF16),
            pltpu.VMEM((F, D), BF16),
            pltpu.VMEM((F, D), BF16),
            pltpu.VMEM((2 * D, D), BF16),
            pltpu.VMEM((D, D), BF16),
            pltpu.VMEM((D, F), BF16),
            pltpu.VMEM((NG, S, LANES), BF16),
            pltpu.VMEM((NG, LANES, S), BF16),
            pltpu.VMEM((H, VR, S), F32),
            pltpu.VMEM((H, VR, S), F32),
            pltpu.VMEM((S, S), F32),
            pltpu.VMEM((8, S), F32),
            pltpu.VMEM((LANES, QS), BF16),
            pltpu.VMEM((S, D), BF16),
            pltpu.SemaphoreType.DMA((7,)),
            pltpu.SemaphoreType.DMA((NRC,)),
            pltpu.SemaphoreType.DMA((S // LANES,)),
        ],
        compiler_params=pltpu.CompilerParams(vmem_limit_bytes=110 * 2 ** 20),
    )(A_x.reshape(S, D), A_wqkv, A_wo, B_w1.T, B_w3.T, B_w2)
    return out.reshape(b, s, d)
```

```python
import jax
import jax.numpy as jnp
from jax.experimental import pallas as pl
from jax.experimental.pallas import tpu as pltpu

BF16 = jnp.bfloat16
F32 = jnp.float32

S = 2048
D = 640
H = 32
DH = D // H
F = 1728
LANES = 128
HG = 6
NG = -(-H // HG)
VR = 24
EPS = 1e-5
QSCALE = (DH ** -0.5) * 1.4426950408889634
NT = (((1,), (1,)), ((), ()))

RC = 512
NRC = S // RC
KC = 256
QS = 256
FC = 896
LNR = 32


def _window_rows(t, g, axis):
    lo = HG * DH * g
    hi = min(lo + LANES, D)
    w = jax.lax.slice_in_dim(t, lo, hi, axis=axis)
    if hi - lo < LANES:
        pad = list(t.shape)
        pad[axis] = lo + LANES - hi
        w = jnp.concatenate([w, jnp.zeros(pad, t.dtype)], axis=axis)
    return w


def _kernel(x_hbm, wqkv_hbm, wo_hbm, w1T_hbm, w3T_hbm, w2_hbm, out_hbm,
            x_v, xn, kraw, wqv_v, wk_v, wo_v, w1T, w3T, w2_v, wqvT, woT, w2T,
            kg, qgT, vpad, opad, sb, msc, qm0, ostage,
            w_sem, x_sem, out_sem):

    def x_cp(r):
        return pltpu.make_async_copy(x_hbm.at[pl.ds(r * RC, RC)], x_v.at[pl.ds(r * RC, RC)], x_sem.at[r])

    def out_cp(r0, i):
        return pltpu.make_async_copy(
            ostage.at[pl.ds(r0, LANES)], out_hbm.at[pl.ds(r0, LANES)], out_sem.at[i])

    wk_cp = pltpu.make_async_copy(wqkv_hbm.at[:, D:2 * D], wk_v, w_sem.at[0])
    wq_cp = pltpu.make_async_copy(wqkv_hbm.at[:, 0:D], wqv_v.at[0:D], w_sem.at[1])
    wv_cp = pltpu.make_async_copy(wqkv_hbm.at[:, 2 * D:3 * D], wqv_v.at[D:2 * D], w_sem.at[2])
    late_cp = [pltpu.make_async_copy(src, dst, w_sem.at[3 + i]) for i, (src, dst) in enumerate(
        ((wo_hbm, wo_v), (w2_hbm, w2_v), (w1T_hbm, w1T), (w3T_hbm, w3T)))]

    def ln_stats(rows):
        xf = x_v[rows, :].astype(F32)
        mu = jnp.mean(xf, axis=-1, keepdims=True)
        xc = xf - mu
        rstd = jax.lax.rsqrt(jnp.mean(xc * xc, axis=-1, keepdims=True) + EPS)
        return xc, mu, rstd

    def ln1(r0, lnr):
        for i in range(RC // lnr):
            rows = pl.ds(r0 + i * lnr, lnr)
            xc, _, rstd = ln_stats(rows)
            xn[rows, :] = (xc * rstd).astype(BF16)

    x_cp(0).start()
    wk_cp.start()
    x_cp(0).wait()
    x_cp(1).start()
    ln1(0, LANES)
    wk_cp.wait()

    def k_chunk(r, carry, transpose_w):
        r0 = pl.multiple_of(r * RC, RC)

        @pl.when(r >= 1)
        def _():
            x_cp(r).wait()

        @pl.when((r >= 1) & (r + 1 < NRC))
        def _():
            x_cp(r + 1).start()

        if not transpose_w:
            @pl.when(r == 0)
            def _():
                wq_cp.start()
                wv_cp.start()

        raw = jnp.dot(x_v[pl.ds(r0, RC), :], wk_v[...], preferred_element_type=F32)
        colsum = jnp.sum(wk_v[...].astype(F32), axis=0, keepdims=True)
        ks = []
        for i in range(RC // LNR):
            _, mu, rstd = ln_stats(pl.ds(r0 + i * LNR, LNR))
            ks.append(((raw[i * LNR:(i + 1) * LNR] - mu * colsum) * rstd).astype(BF16))
        kraw[pl.ds(r0, RC), :] = jnp.concatenate(ks, axis=0)
        if transpose_w:
            wr = pl.ds(pl.multiple_of((r - NRC // 2) * D, D), D)
            wqvT[wr, :] = wqv_v[wr, :].T
        return carry

    jax.lax.fori_loop(0, NRC // 2, lambda r, c: k_chunk(r, c, False), 0)
    wq_cp.wait()
    wv_cp.wait()
    jax.lax.fori_loop(NRC // 2, NRC, lambda r, c: k_chunk(r, c, True), 0)
    for c in late_cp:
        c.start()

    def qv_chunk(r, carry):
        r0 = pl.multiple_of(r * RC, RC)
        cols = pl.ds(r0, RC)
        qv = jax.lax.dot_general(wqvT[...], xn[cols, :], NT, preferred_element_type=F32)
        for i in range(RC // LNR):
            rows = pl.ds(r0 + i * LNR, LNR)
            k = kraw[rows, :]
            for g in range(NG):
                kg[g, rows, :] = _window_rows(k, g, 1)
        qT = qv[0:D] * QSCALE
        for g in range(NG):
            qgT[g, :, cols] = _window_rows(qT, g, 0).astype(BF16)
        vT = qv[D:2 * D].astype(BF16).astype(F32)
        vT = jnp.concatenate([vT, jnp.zeros((8, RC), F32)], axis=0)
        row = jax.lax.broadcasted_iota(jnp.int32, (VR, RC), 0)
        fill = jnp.where(row == DH, 1.0, 0.0).astype(F32)
        for h in range(H):
            vpad[h, :, cols] = jnp.where(row < DH, vT[DH * h:DH * h + VR], fill)
        ln1(pl.multiple_of(jnp.minimum(r + 1, NRC - 1) * RC, RC), LNR)
        return carry

    jax.lax.fori_loop(0, NRC, qv_chunk, 0)

    nqs = S // QS
    nkc = S // KC

    def masked_q(g, lo, j):
        row = jax.lax.broadcasted_iota(jnp.int32, (LANES, QS), 0)
        q = qgT[g, :, j * QS:(j + 1) * QS]
        return jnp.where((row >= lo) & (row < lo + DH), q, jnp.zeros_like(q))

    def score_chunk(g, qm, c, j, mx):
        s = jnp.dot(kg[g, c * KC:(c + 1) * KC, :], qm, preferred_element_type=F32)
        sb[c * KC:(c + 1) * KC, j * QS:(j + 1) * QS] = s
        bm = jnp.max(s.reshape(KC // 8, 8, QS), axis=0)
        return bm if mx is None else jnp.maximum(mx, bm)

    def row_max(j):
        m = jnp.max(msc[:, j * QS:(j + 1) * QS], axis=0, keepdims=True)
        return jnp.broadcast_to(m, (8, QS))

    def probs(c, j, m8):
        s = sb[c * KC:(c + 1) * KC, j * QS:(j + 1) * QS]
        return jnp.exp2(s.reshape(KC // 8, 8, QS) - m8[None]).reshape(KC, QS).astype(BF16)

    def pv_chunk(h, c, p, o):
        d = jnp.dot(vpad[h, :, c * KC:(c + 1) * KC], p, preferred_element_type=F32)
        return d if o is None else o + d

    def step(h, carry):
        g, lo = carry
        m_cur = [row_max(j) for j in range(nqs)]
        m_nxt = []
        for j in range(nqs):
            qm = qm0[...] if j == 0 else masked_q(g, lo, j)
            mx, o = None, None
            for c in range(nkc):
                p = probs(c, j, m_cur[j])
                mx = score_chunk(g, qm, c, j, mx)
                o = pv_chunk(h, c, p, o)
            opad[h, :, j * QS:(j + 1) * QS] = o
            m_nxt.append(mx)
        for j in range(nqs):
            msc[:, j * QS:(j + 1) * QS] = m_nxt[j]
        wrap = lo + DH >= HG * DH
        g2, lo2 = jnp.where(wrap, g + 1, g), jnp.where(wrap, 0, lo + DH)
        qm0[...] = masked_q(jnp.minimum(g2, NG - 1), lo2, 0)
        return g2, lo2

    for j in range(nqs):
        qm = masked_q(0, 0, j)
        mx = None
        for c in range(nkc):
            mx = score_chunk(0, qm, c, j, mx)
        msc[:, j * QS:(j + 1) * QS] = mx
    qm0[...] = masked_q(0, DH, 0)

    jax.lax.fori_loop(0, H - 1, step, (jnp.int32(0), jnp.int32(DH)))

    for c in late_cp:
        c.wait()
    tpieces = [(wo_v, woT, a, LANES) for a in range(0, D, LANES)]
    tpieces += [(w2_v, w2T, a, min(LANES, F - a)) for a in range(0, F, LANES)]
    n = 0
    for j in range(nqs):
        m8 = row_max(j)
        o = None
        for c in range(nkc):
            o = pv_chunk(H - 1, c, probs(c, j, m8), o)
            if n % 3 == 1 and tpieces:
                src, dst, a, w = tpieces.pop(0)
                dst[:, a:a + w] = src[a:a + w, :].T
            n += 1
        opad[H - 1, :, j * QS:(j + 1) * QS] = o
    assert not tpieces

    fchunks = [(f0, min(FC, F - f0)) for f0 in range(0, F, FC)]

    def mlp_chunk(r, carry):
        r0 = pl.multiple_of(r * RC, RC)
        cols = pl.ds(r0, RC)
        pieces = []
        for h in range(H):
            oh = opad[h, :, cols]
            pieces.append(oh[0:DH] * (1.0 / oh[DH:DH + 1]))
        oT = jnp.concatenate(pieces, axis=0).astype(BF16)
        hT = x_v[cols, :].astype(F32).T + jnp.dot(woT[...], oT, preferred_element_type=F32)
        mu = jnp.mean(hT, axis=0, keepdims=True)
        hc = hT - mu
        var = jnp.mean(hc * hc, axis=0, keepdims=True)
        hn = (hc * jax.lax.rsqrt(var + EPS)).astype(BF16)

        def gate_up(i):
            f0, fw = fchunks[i]
            w = jnp.concatenate([w1T[f0:f0 + fw, :], w3T[f0:f0 + fw, :]], axis=0)
            gu = jnp.dot(w, hn, preferred_element_type=F32)
            return gu[0:fw], gu[fw:2 * fw]

        acc = hT
        cur = gate_up(0)
        for i, (f0, fw) in enumerate(fchunks):
            nxt = gate_up(i + 1) if i + 1 < len(fchunks) else None
            g, u = cur
            act = (g * jax.nn.sigmoid(g) * u).astype(BF16)
            acc = acc + jnp.dot(w2T[:, f0:f0 + fw], act, preferred_element_type=F32)
            cur = nxt
        for i in range(RC // LANES):
            rr = pl.multiple_of(r0 + i * LANES, LANES)
            ostage[pl.ds(rr, LANES), :] = acc[:, i * LANES:(i + 1) * LANES].T.astype(BF16)
            out_cp(rr, r * (RC // LANES) + i).start()
        return carry

    jax.lax.fori_loop(0, NRC, mlp_chunk, 0)
    for i in range(S // LANES):
        out_cp(i * LANES, i).wait()


@jax.jit
def pallas_sequential_preLN__softmax_full_mha__glu_gated_swiglu__prompt_kernel(
    A_x: jax.Array,
    A_wqkv: jax.Array,
    A_wo: jax.Array,
    B_x: jax.Array,
    B_w1: jax.Array,
    B_w3: jax.Array,
    B_w2: jax.Array,
):
    del B_x
    b, s, d = A_x.shape
    assert (b, s, d) == (1, S, D) and B_w1.shape == (D, F)
    hbm = pl.BlockSpec(memory_space=pltpu.MemorySpace.HBM)
    out = pl.pallas_call(
        _kernel,
        out_shape=jax.ShapeDtypeStruct((S, D), A_x.dtype),
        in_specs=[hbm] * 6,
        out_specs=hbm,
        scratch_shapes=[
            pltpu.VMEM((S, D), BF16),
            pltpu.VMEM((S, D), BF16),
            pltpu.VMEM((S, D), BF16),
            pltpu.VMEM((2 * D, D), BF16),
            pltpu.VMEM((D, D), BF16),
            pltpu.VMEM((D, D), BF16),
            pltpu.VMEM((F, D), BF16),
            pltpu.VMEM((F, D), BF16),
            pltpu.VMEM((F, D), BF16),
            pltpu.VMEM((2 * D, D), BF16),
            pltpu.VMEM((D, D), BF16),
            pltpu.VMEM((D, F), BF16),
            pltpu.VMEM((NG, S, LANES), BF16),
            pltpu.VMEM((NG, LANES, S), BF16),
            pltpu.VMEM((H, VR, S), F32),
            pltpu.VMEM((H, VR, S), F32),
            pltpu.VMEM((S, S), F32),
            pltpu.VMEM((8, S), F32),
            pltpu.VMEM((LANES, QS), BF16),
            pltpu.VMEM((S, D), BF16),
            pltpu.SemaphoreType.DMA((7,)),
            pltpu.SemaphoreType.DMA((NRC,)),
            pltpu.SemaphoreType.DMA((S // LANES,)),
        ],
        compiler_params=pltpu.CompilerParams(vmem_limit_bytes=110 * 2 ** 20),
    )(A_x.reshape(S, D), A_wqkv, A_wo, B_w1.T, B_w3.T, B_w2)
    return out.reshape(b, s, d)
```
